```python
import os as _os
_os.environ.setdefault("JAX_PLATFORMS", "cpu")
import jax
import jax.numpy as jnp

def _softmax(x, axis=-1):
    return jax.nn.softmax(x, axis=axis)
def _gelu(x):
    return jax.nn.gelu(x, approximate=True)
def _silu(x):
    return jax.nn.silu(x)
def _sigmoid(x):
    return jax.nn.sigmoid(x)
def _layernorm(x, axis=-1, eps=1e-5):
    m = jnp.mean(x, axis=axis, keepdims=True)
    v = jnp.var(x, axis=axis, keepdims=True)
    return (x - m) / jnp.sqrt(v + eps)
def _scatter_add(tgt, idx, src, axis=0):
    return tgt.at[idx].add(src)
def _segment_sum(src, seg, n):
    return jax.ops.segment_sum(src, seg, n)
class _Rng:
    def __init__(self, key):
        self._k = key
    def _next(self):
        self._k, sub = jax.random.split(self._k)
        return sub
    def normal(self, shape):
        return jax.random.normal(self._next(), shape, dtype=jnp.bfloat16)
    def randint(self, lo, hi, shape):
        return jax.random.randint(self._next(), shape, lo, hi, dtype=jnp.int32)
    def uniform(self, shape, lo=0.0, hi=1.0):
        return jax.random.uniform(self._next(), shape, jnp.bfloat16, lo, hi)
    def permutation(self, n):
        return jax.random.permutation(self._next(), n)


kernel_name = 'gated_mix__compressed_kv_cla__linear_attn_block__prompt'

def setup_inputs():
    _rng = _Rng(jax.random.key(int.from_bytes(__import__("os").urandom(4), "little")))
    _w = (lambda a: (lambda t: t.astype(jnp.bfloat16) if jnp.issubdtype(t.dtype, jnp.floating) else t)(jnp.asarray(a)))
    def _A_setup():
        B, H, Sq, Sk, D, M = 1, 16, 2048, 2048, 256, 448
        Dc = 4 * D
        return {
            "x": _w((lambda *s: _rng.normal(s) * 0.05)(B, Sq, M)),
            "c_kv": _w((lambda *s: _rng.normal(s) * 0.8)(B, Sk, Dc)),
            "w_q": _w((lambda *s: _rng.normal(s) * 3.2)(M, H, D) * (M ** -0.5)),
            "w_uk": _w((lambda *s: _rng.normal(s) * 3.2)(Dc, H, D) * (Dc ** -0.5)),
            "w_uv": _w((lambda *s: _rng.normal(s) * 0.8)(Dc, H, D) * (Dc ** -0.5)),
            "w_o": _w((lambda *s: _rng.normal(s) * 0.8)(H, D, M) * ((H * D) ** -0.5)),
        }
    _A_in = _A_setup()

    def _B_setup():
        B, S, D = 1, 2048, 448
        return {
            "x": _w((lambda *s: _rng.normal(s) * 0.05)(B, S, D)),
            "wqkv": _w((lambda *s: _rng.normal(s) * 1.6)(D, 3 * D)),
            "wo": _w((lambda *s: _rng.normal(s) * 0.4)(D, D)),
        }
    _B_in = _B_setup()

    return {
        "A_x": _A_in["x"],
        "A_c_kv": _A_in["c_kv"],
        "A_w_q": _A_in["w_q"],
        "A_w_uk": _A_in["w_uk"],
        "A_w_uv": _A_in["w_uv"],
        "A_w_o": _A_in["w_o"],
        "B_x": _B_in["x"],
        "B_wqkv": _B_in["wqkv"],
        "B_wo": _B_in["wo"],
        "gate_w": _w((lambda *s: _rng.normal(s) * 0.05)(448) * 16.0),
    }

def reference(A_x, A_c_kv, A_w_q, A_w_uk, A_w_uv, A_w_o, B_x, B_wqkv, B_wo, gate_w):
    def _A_ref(x, c_kv, w_q, w_uk, w_uv, w_o):
        B, Sq, M = x.shape[0], x.shape[1], x.shape[2]
        Sk = c_kv.shape[1]
        H, D = w_q.shape[1], w_q.shape[2]
        q = jnp.einsum("bqm,mhd->bhqd", x, w_q)
        k = jnp.einsum("bkc,chd->bhkd", c_kv, w_uk)
        v = jnp.einsum("bkc,chd->bhkd", c_kv, w_uv)
        scores = jnp.einsum("bhqd,bhkd->bhqk", q, k) * (D ** -0.5)
        off = Sk - Sq
        qi = jnp.arange(Sq)[:, None]
        kj = jnp.arange(Sk)[None, :]
        cmask = kj <= (qi + off)
        scores = jnp.where(cmask[None, None], scores, -1e9)
        p = _softmax(scores, axis=-1)
        ctx = jnp.einsum("bhqk,bhkd->bhqd", p, v)
        return jnp.einsum("bhqd,hdm->bqm", ctx, w_o)

    def _B_ref(x, wqkv, wo):
        B, S, D = x.shape
        H = 16; Dh = D // H
        qkv = (lambda x, *d: x.transpose(*d))((x @ wqkv).reshape(B, S, 3, H, Dh), 2, 0, 3, 1, 4)
        q, k, v = qkv[0], qkv[1], qkv[2]
        phi = lambda t: jnp.where(t > 0, t + 1, jnp.exp(t)) + 1e-6
        pq, pk = phi(q), phi(k)
        kv = jnp.einsum("bhsd,bhse->bhde", pk, v)
        z = jnp.einsum("bhsd->bhd", pk)
        num = jnp.einsum("bhqd,bhde->bhqe", pq, kv)
        den = jnp.einsum("bhqd,bhd->bhq", pq, z)[..., None] + 1e-6
        o = num / den
        return (lambda x, *d: x.transpose(*d))(o, 0, 2, 1, 3).reshape(B, S, D) @ wo

    x = A_x
    g = _sigmoid((x * gate_w).sum(-1, keepdims=True))
    a = _A_ref(x, A_c_kv, A_w_q, A_w_uk, A_w_uv, A_w_o)
    b = _B_ref(x, B_wqkv, B_wo)
    return g * a + (1 - g) * b
```

```python
import numpy as np
import jax
import jax.numpy as jnp
from jax import lax
import jax.experimental.pallas as pl
import jax.experimental.pallas.tpu as pltpu

S = 2048
M = 448
H = 16
D = 256
DC = 1024
DH = 28
TQ = 256
HT = TQ // 2
NQ = S // TQ
CB = 512
NCB = S // CB
WCH = 4
NT_DIMS = (((1,), (1,)), ((), ()))
TN_DIMS = (((0,), (0,)), ((), ()))
F32 = jnp.float32
BF16 = jnp.bfloat16
LOG2E = 1.4426950408889634
NEG = -1e30


def _dot(a, b):
    return jnp.dot(a, b, preferred_element_type=F32)


def _dot_nt(a, b):
    return lax.dot_general(a, b, NT_DIMS, preferred_element_type=F32)


def _dot_tn(a, b):
    return lax.dot_general(a, b, TN_DIMS, preferred_element_type=F32)


def _phi(t):
    return jnp.where(t > 0, t + 1.0, jnp.exp(t)) + 1e-6


def _relayout(src_ref, dst_ref, base, nrows):
    for t in range(0, nrows, 16):
        m0 = base + t
        if not isinstance(m0, int):
            m0 = pl.multiple_of(m0, 16)
        dst_ref[:, pl.ds(m0, 16), :] = jnp.swapaxes(src_ref[pl.ds(m0, 16)], 0, 1)


def _scores(i, q_s, k_s):
    q = q_s[pl.ds(i * TQ, TQ), :]
    n = i * TQ + HT
    s = _dot_nt(q, k_s[pl.ds(0, n), :])
    s_l = _dot_nt(q[HT:], k_s[pl.ds(n, HT), :])
    r = lax.broadcasted_iota(jnp.int32, (HT, HT), 0)
    c = lax.broadcasted_iota(jnp.int32, (HT, HT), 1)
    s_l = jnp.where(c <= r, s_l, NEG)
    r2 = lax.broadcasted_iota(jnp.int32, (TQ, HT), 0)
    c2 = lax.broadcasted_iota(jnp.int32, (TQ, HT), 1)
    s_d = jnp.where(c2 <= r2, s[:, i * TQ:], NEG)
    s = jnp.concatenate([s[:, :i * TQ], s_d], axis=1) if i > 0 else s_d
    m = jnp.max(s, axis=1, keepdims=True)
    m_b = jnp.maximum(m[HT:], jnp.max(s_l, axis=1, keepdims=True))
    m = jnp.concatenate([m[:HT], m_b], axis=0)
    p = jnp.exp2(s - m)
    p_l = jnp.exp2(s_l - m_b)
    l = jnp.sum(p, axis=1, keepdims=True)
    l_b = l[HT:] + jnp.sum(p_l, axis=1, keepdims=True)
    l = jnp.concatenate([l[:HT], l_b], axis=0)
    return p.astype(BF16), p_l.astype(BF16), l


def _context(i, st, v_s):
    p, p_l, l = st
    n = i * TQ + HT
    acc = _dot(p, v_s[pl.ds(0, n), :])
    acc_b = acc[HT:] + _dot(p_l, v_s[pl.ds(n, HT), :])
    acc = jnp.concatenate([acc[:HT], acc_b], axis=0)
    return (acc * (1.0 / l)).astype(BF16)


def kernel(axT_hbm, ckv_hbm, wq_hbm, wuk_hbm, wuv_hbm, woT_hbm, wqkv_hbm, bwo_hbm, gate_ref,
           outT_ref,
           axT, ckv, wq, wuk, wuv, woT, wqkv, bwo,
           x_s, wqT, wukT, wuvT, q_s, k_s, v_s, pq_s, g_s, acc_s, wqkT, G_s, z_s, wp_s, inv_s, sems):
    KC = DC // WCH
    cp_wqkv = pltpu.make_async_copy(wqkv_hbm, wqkv, sems.at[1])
    cp_ckv = pltpu.make_async_copy(ckv_hbm, ckv, sems.at[2])
    cp_wq = pltpu.make_async_copy(wq_hbm, wq, sems.at[3])
    cp_bwo = pltpu.make_async_copy(bwo_hbm, bwo, sems.at[4])
    cp_wo = pltpu.make_async_copy(woT_hbm, woT, sems.at[5])

    def cp_wuk(c):
        rows = pl.ds(c * KC, KC)
        return pltpu.make_async_copy(wuk_hbm.at[rows], wuk.at[rows], sems.at[6 + c])

    def cp_wuv(c):
        rows = pl.ds(c * KC, KC)
        return pltpu.make_async_copy(wuv_hbm.at[rows], wuv.at[rows], sems.at[6 + WCH + c])

    XC = NCB
    def cp_x(c):
        cols = pl.ds(c * (S // XC), S // XC)
        return pltpu.make_async_copy(axT_hbm.at[:, cols], axT.at[:, cols], sems.at[6 + 2 * WCH + c])

    for cp in [cp_wqkv, cp_x(0), cp_bwo, *[cp_x(c) for c in range(1, XC)], *[cp_wuk(c) for c in range(WCH)], cp_ckv, cp_wq,
               *[cp_wuv(c) for c in range(WCH)], cp_wo]:
        cp.start()

    qscale = (D ** -0.5) * LOG2E

    def relayout_loop(src, dst, base, nrows, step=64):
        def body(i, carry):
            _relayout(src, dst, base + i * step, step)
            return carry
        lax.fori_loop(0, nrows // step, body, 0)

    cp_wqkv.wait()
    wqkT[0:2 * M, :] = wqkv[:, 0:2 * M].T
    rid16 = lax.broadcasted_iota(jnp.int32, (16, M), 0)
    wqkT[2 * M:2 * M + 16, :] = jnp.where(rid16 == 0, jnp.broadcast_to(gate_ref[...], (16, M)), 0).astype(BF16)
    G_s[...] = jnp.zeros_like(G_s)
    z_s[...] = jnp.zeros_like(z_s)

    def b1_body(c, carry):
        cp_x(c).wait()
        cols = pl.ds(pl.multiple_of(c * CB, CB), CB)
        xT = axT[:, cols]
        pq_s[:, cols] = _phi(_dot(wqkT[0:M, :], xT)).astype(BF16)
        kg = _dot(wqkT[M:2 * M + 16, :], xT)
        g_s[:, cols] = jnp.broadcast_to(jax.nn.sigmoid(kg[M:M + 1]), (8, CB))
        pk = _phi(kg[:M])
        zp = pk[:, 0:128]
        for t in range(1, CB // 128):
            zp = zp + pk[:, t * 128:(t + 1) * 128]
        z_s[...] += zp
        G_s[...] += _dot_nt(pk.astype(BF16), xT)
        return carry

    lax.fori_loop(0, NCB, b1_body, 0)

    for c in range(WCH):
        cp_wuk(c).wait()
    relayout_loop(wuk, wukT, 0, DC)

    cp_bwo.wait()
    cp_ckv.wait()
    k_s[...] = _dot(ckv[...], wukT[0]).astype(BF16)
    rr = lax.broadcasted_iota(jnp.int32, (M, M), 0) // DH
    cc = lax.broadcasted_iota(jnp.int32, (M, M), 1) // DH
    KV = jnp.where(rr == cc, _dot(G_s[...].astype(BF16), wqkv[:, 2 * M:3 * M]), 0.0)
    WpT = _dot(KV.astype(BF16), bwo[...]).astype(BF16).T
    zc = jnp.sum(z_s[...], axis=1, keepdims=True)
    z_row = jnp.broadcast_to(zc, (M, 128)).T[0:H, :]
    hh = lax.broadcasted_iota(jnp.int32, (H, M), 0)
    hc = lax.broadcasted_iota(jnp.int32, (H, M), 1) // DH
    z_lhs = jnp.where(hh == hc, z_row, 0.0).astype(BF16)
    wp_s[...] = WpT
    GR = 4 * DH
    rid = lax.broadcasted_iota(jnp.int32, (GR, CB), 0)
    inv_s[...] = 1.0 / (_dot(z_lhs, pq_s[...]) + 1e-6)

    def b2_body(c, carry):
        c0 = pl.multiple_of(c * CB, CB)
        cols = pl.ds(c0, CB)
        x_s[cols, :] = axT[:, cols].T
        pq = pq_s[:, cols]
        inv = inv_s[:, cols]
        parts = []
        for gi in range(M // GR):
            e = jnp.where(rid < DH, inv[4 * gi:4 * gi + 1],
                          jnp.where(rid < 2 * DH, inv[4 * gi + 1:4 * gi + 2],
                                    jnp.where(rid < 3 * DH, inv[4 * gi + 2:4 * gi + 3],
                                              inv[4 * gi + 3:4 * gi + 4])))
            parts.append((pq[gi * GR:(gi + 1) * GR].astype(F32) * e).astype(BF16))
        pqn = jnp.concatenate(parts, axis=0)
        acc_s[:, cols] = (1.0 - g_s[0:1, cols]) * _dot(wp_s[...], pqn)
        return carry

    lax.fori_loop(0, NCB, b2_body, 0)

    cp_wq.wait()
    relayout_loop(wq, wqT, 0, M)
    q_s[...] = (_dot(x_s[...], wqT[0]) * qscale).astype(BF16)
    for c in range(WCH):
        cp_wuv(c).wait()
        relayout_loop(wuv, wuvT, c * KC, KC)
    cp_wo.wait()

    def head_body(h, carry):
        v_s[...] = _dot(ckv[...], wuvT[h]).astype(BF16)
        w_o = woT[h]

        def out_proj(i, ctx):
            cols = pl.ds(i * TQ, TQ)
            new = acc_s[:, cols] + g_s[0:1, cols] * _dot_nt(w_o, ctx)
            acc_s[:, cols] = new
            outT_ref[:, cols] = new.astype(outT_ref.dtype)

        pend, opend = [], []
        for i in range(NQ - 1, -1, -1):
            pend.append((i, _scores(i, q_s, k_s)))
            if len(pend) > 1:
                pi, st = pend.pop(0)
                opend.append((pi, _context(pi, st, v_s)))
                if len(opend) > 1:
                    out_proj(*opend.pop(0))
        pi, st = pend.pop(0)
        opend.append((pi, _context(pi, st, v_s)))
        for o in opend:
            out_proj(*o)

        @pl.when(h < H - 1)
        def _():
            k_s[...] = _dot(ckv[...], wukT[h + 1]).astype(BF16)
            q_s[...] = (_dot(x_s[...], wqT[h + 1]) * qscale).astype(BF16)

        return carry

    lax.fori_loop(0, H, head_body, 0)


@jax.jit
def pallas_gated_mix__compressed_kv_cla__linear_attn_block__prompt_kernel(
    A_x: jax.Array,
    A_c_kv: jax.Array,
    A_w_q: jax.Array,
    A_w_uk: jax.Array,
    A_w_uv: jax.Array,
    A_w_o: jax.Array,
    B_x: jax.Array,
    B_wqkv: jax.Array,
    B_wo: jax.Array,
    gate_w: jax.Array,
):
    del B_x
    hbm = pl.BlockSpec(memory_space=pltpu.HBM)
    outT = pl.pallas_call(
        kernel,
        out_shape=jax.ShapeDtypeStruct((M, S), BF16),
        in_specs=[hbm] * 8 + [pl.BlockSpec((1, M), lambda: (0, 0))],
        out_specs=pl.BlockSpec((M, S), lambda: (0, 0)),
        scratch_shapes=[
            pltpu.VMEM((M, S), BF16),
            pltpu.VMEM((S, DC), BF16),
            pltpu.VMEM((M, H, D), BF16),
            pltpu.VMEM((DC, H, D), BF16),
            pltpu.VMEM((DC, H, D), BF16),
            pltpu.VMEM((H, M, D), BF16),
            pltpu.VMEM((M, 3 * M), BF16),
            pltpu.VMEM((M, M), BF16),
            pltpu.VMEM((S, M), BF16),
            pltpu.VMEM((H, M, D), BF16),
            pltpu.VMEM((H, DC, D), BF16),
            pltpu.VMEM((H, DC, D), BF16),
            pltpu.VMEM((S, D), BF16),
            pltpu.VMEM((S, D), BF16),
            pltpu.VMEM((S, D), BF16),
            pltpu.VMEM((M, S), BF16),
            pltpu.VMEM((8, S), F32),
            pltpu.VMEM((M, S), F32),
            pltpu.VMEM((2 * M + 16, M), BF16),
            pltpu.VMEM((M, M), F32),
            pltpu.VMEM((M, 128), F32),
            pltpu.VMEM((M, M), BF16),
            pltpu.VMEM((H, S), F32),
            pltpu.SemaphoreType.DMA((6 + 2 * WCH + NCB,)),
        ],
        compiler_params=pltpu.CompilerParams(vmem_limit_bytes=110 * 2**20),
        name="gmk",
    )(A_x[0].T, A_c_kv[0], A_w_q, A_w_uk, A_w_uv, A_w_o.transpose(0, 2, 1),
      B_wqkv, B_wo, gate_w.reshape(1, M))
    return outT.T[None]
```

```python
import functools
import numpy as np
import jax
import jax.numpy as jnp
from jax import lax
import jax.experimental.pallas as pl
import jax.experimental.pallas.tpu as pltpu

S = 2048
M = 448
H = 16
D = 256
DC = 1024
DH = 28
TQ = 256
HT = TQ // 2
NQ = S // TQ
CB = 512
NCB = S // CB
WCH = 4
NT_DIMS = (((1,), (1,)), ((), ()))
TN_DIMS = (((0,), (0,)), ((), ()))
F32 = jnp.float32
BF16 = jnp.bfloat16
LOG2E = 1.4426950408889634
NEG = -1e9 * LOG2E


def _dot(a, b):
    return jnp.dot(a, b, preferred_element_type=F32)


def _dot_nt(a, b):
    return lax.dot_general(a, b, NT_DIMS, preferred_element_type=F32)


def _dot_tn(a, b):
    return lax.dot_general(a, b, TN_DIMS, preferred_element_type=F32)


def _phi(t):
    return jnp.where(t > 0, t + 1.0, jnp.exp(t)) + 1e-6


def _relayout(src_ref, dst_ref, base, nrows):
    for t in range(0, nrows, 16):
        m0 = base + t
        if not isinstance(m0, int):
            m0 = pl.multiple_of(m0, 16)
        dst_ref[:, pl.ds(m0, 16), :] = jnp.swapaxes(src_ref[pl.ds(m0, 16)], 0, 1)


def _scores(i, q_s, k_s):
    q = q_s[pl.ds(i * TQ, TQ), :]
    n = i * TQ + HT
    s = _dot_nt(q, k_s[pl.ds(0, n), :])
    s_l = _dot_nt(q[HT:], k_s[pl.ds(n, HT), :])
    r = lax.broadcasted_iota(jnp.int32, (HT, HT), 0)
    c = lax.broadcasted_iota(jnp.int32, (HT, HT), 1)
    s_l = jnp.where(c <= r, s_l, NEG)
    r2 = lax.broadcasted_iota(jnp.int32, (TQ, HT), 0)
    c2 = lax.broadcasted_iota(jnp.int32, (TQ, HT), 1)
    s_d = jnp.where(c2 <= r2, s[:, i * TQ:], NEG)
    s = jnp.concatenate([s[:, :i * TQ], s_d], axis=1) if i > 0 else s_d
    m = jnp.max(s, axis=1, keepdims=True)
    m_b = jnp.maximum(m[HT:], jnp.max(s_l, axis=1, keepdims=True))
    m = jnp.concatenate([m[:HT], m_b], axis=0)
    p = jnp.exp2(s - m)
    p_l = jnp.exp2(s_l - m_b)
    l = jnp.sum(p, axis=1, keepdims=True)
    l_b = l[HT:] + jnp.sum(p_l, axis=1, keepdims=True)
    l = jnp.concatenate([l[:HT], l_b], axis=0)
    return p.astype(BF16), p_l.astype(BF16), l


def _context(i, st, v_s):
    p, p_l, l = st
    n = i * TQ + HT
    acc = _dot(p, v_s[pl.ds(0, n), :])
    acc_b = acc[HT:] + _dot(p_l, v_s[pl.ds(n, HT), :])
    acc = jnp.concatenate([acc[:HT], acc_b], axis=0)
    return (acc * (1.0 / l)).astype(BF16)


def kernel(axT_hbm, ckv_hbm, wq_hbm, wuk_hbm, wuv_hbm, woT_hbm, wqkv_hbm, bwo_hbm, gate_ref,
           outT_ref,
           axT, ckv, wq, wuk, wuv, woT, wqkv, bwo,
           x_s, wqT, wukT, wuvT, q_s, k_s, v_s, pq_s, g_s, acc_s, wqkT, G_s, z_s, wp_s, inv_s, sems):
    KC = DC // WCH
    cp_wqk = pltpu.make_async_copy(wqkv_hbm.at[:, 0:2 * M], wqkv.at[:, 0:2 * M], sems.at[1])
    cp_wv = pltpu.make_async_copy(wqkv_hbm.at[:, 2 * M:3 * M], wqkv.at[:, 2 * M:3 * M], sems.at[0])
    cp_ckv = pltpu.make_async_copy(ckv_hbm, ckv, sems.at[2])
    cp_wq = pltpu.make_async_copy(wq_hbm, wq, sems.at[3])
    cp_bwo = pltpu.make_async_copy(bwo_hbm, bwo, sems.at[4])
    cp_wo = pltpu.make_async_copy(woT_hbm, woT, sems.at[5])

    def cp_wuk(c):
        rows = pl.ds(c * KC, KC)
        return pltpu.make_async_copy(wuk_hbm.at[rows], wuk.at[rows], sems.at[6 + c])

    def cp_wuv(c):
        rows = pl.ds(c * KC, KC)
        return pltpu.make_async_copy(wuv_hbm.at[rows], wuv.at[rows], sems.at[6 + WCH + c])

    XC = NCB
    def cp_x(c):
        cols = pl.ds(c * (S // XC), S // XC)
        return pltpu.make_async_copy(axT_hbm.at[:, cols], axT.at[:, cols], sems.at[6 + 2 * WCH + c])

    for cp in [cp_wqk, *[cp_x(c) for c in range(XC)], cp_wv, cp_bwo, *[cp_wuk(c) for c in range(WCH)], cp_ckv, cp_wq,
               *[cp_wuv(c) for c in range(WCH)], cp_wo]:
        cp.start()

    qscale = (D ** -0.5) * LOG2E

    def relayout_loop(src, dst, base, nrows, step=64):
        def body(i, carry):
            _relayout(src, dst, base + i * step, step)
            return carry
        lax.fori_loop(0, nrows // step, body, 0)

    cp_wqk.wait()
    wqkT[0:2 * M, :] = wqkv[:, 0:2 * M].T
    rid16 = lax.broadcasted_iota(jnp.int32, (16, M), 0)
    wqkT[2 * M:2 * M + 16, :] = jnp.where(rid16 == 0, jnp.broadcast_to(gate_ref[...].reshape(1, M), (16, M)), 0).astype(BF16)
    G_s[...] = jnp.zeros_like(G_s)
    z_s[...] = jnp.zeros_like(z_s)

    def b1_body(c, carry):
        cp_x(c).wait()
        cols = pl.ds(pl.multiple_of(c * CB, CB), CB)
        xT = axT[:, cols]
        pq_s[:, cols] = _phi(_dot(wqkT[0:M, :], xT)).astype(BF16)
        kg = _dot(wqkT[M:2 * M + 16, :], xT)
        g_s[:, cols] = jnp.broadcast_to(jax.nn.sigmoid(kg[M:M + 1]), (8, CB))
        pk = _phi(kg[:M])
        zp = pk[:, 0:128]
        for t in range(1, CB // 128):
            zp = zp + pk[:, t * 128:(t + 1) * 128]
        z_s[...] += zp
        G_s[...] += _dot_nt(pk.astype(BF16), xT)
        return carry

    lax.fori_loop(0, NCB, b1_body, 0)

    for c in range(WCH):
        cp_wuk(c).wait()
    relayout_loop(wuk, wukT, 0, DC)

    cp_wv.wait()
    cp_bwo.wait()
    cp_ckv.wait()
    k_s[...] = _dot(ckv[...], wukT[0]).astype(BF16)
    Gb = G_s[...].astype(BF16)
    wp_rows = []
    for r0 in range(0, M, 128):
        r1 = min(r0 + 128, M)
        c0 = (r0 // DH * DH) // 128 * 128
        c1 = min(-(-(-(-r1 // DH) * DH) // 128) * 128, M)
        rr = (lax.broadcasted_iota(jnp.int32, (r1 - r0, c1 - c0), 0) + r0) // DH
        cc = (lax.broadcasted_iota(jnp.int32, (r1 - r0, c1 - c0), 1) + c0) // DH
        kv = jnp.where(rr == cc, _dot(Gb[r0:r1], wqkv[:, 2 * M + c0:2 * M + c1]), 0.0)
        wp_rows.append(_dot(kv.astype(BF16), bwo[c0:c1, :]))
    WpT = jnp.concatenate(wp_rows, axis=0).astype(BF16).T
    zc = jnp.sum(z_s[...], axis=1, keepdims=True)
    z_row = jnp.broadcast_to(zc, (M, 128)).T[0:H, :]
    hh = lax.broadcasted_iota(jnp.int32, (H, M), 0)
    hc = lax.broadcasted_iota(jnp.int32, (H, M), 1) // DH
    z_lhs = jnp.where(hh == hc, z_row, 0.0).astype(BF16)
    wp_s[...] = WpT
    GR = 4 * DH
    rid = lax.broadcasted_iota(jnp.int32, (GR, CB), 0)
    inv_s[...] = 1.0 / (_dot(z_lhs, pq_s[...]) + 1e-6)

    def b2_body(c, carry):
        c0 = pl.multiple_of(c * CB, CB)
        cols = pl.ds(c0, CB)
        x_s[cols, :] = axT[:, cols].T
        pq = pq_s[:, cols]
        inv = inv_s[:, cols]
        parts = []
        for gi in range(M // GR):
            e = jnp.where(rid < DH, inv[4 * gi:4 * gi + 1],
                          jnp.where(rid < 2 * DH, inv[4 * gi + 1:4 * gi + 2],
                                    jnp.where(rid < 3 * DH, inv[4 * gi + 2:4 * gi + 3],
                                              inv[4 * gi + 3:4 * gi + 4])))
            parts.append((pq[gi * GR:(gi + 1) * GR].astype(F32) * e).astype(BF16))
        pqn = jnp.concatenate(parts, axis=0)
        acc_s[:, cols] = (1.0 - g_s[0:1, cols]) * _dot(wp_s[...], pqn)
        return carry

    lax.fori_loop(0, NCB, b2_body, 0)

    cp_wq.wait()
    relayout_loop(wq, wqT, 0, M)
    q_s[...] = (_dot(x_s[...], wqT[0]) * qscale).astype(BF16)
    for c in range(WCH):
        cp_wuv(c).wait()
        relayout_loop(wuv, wuvT, c * KC, KC)
    cp_wo.wait()

    def head_body(h, carry):
        v_s[...] = _dot(ckv[...], wuvT[h]).astype(BF16)
        w_o = woT[h]

        def out_proj(i, ctx):
            cols = pl.ds(i * TQ, TQ)
            new = acc_s[:, cols] + g_s[0:1, cols] * _dot_nt(w_o, ctx)
            acc_s[:, cols] = new
            outT_ref[:, cols] = new.astype(outT_ref.dtype)

        pend, opend = [], []
        for i in range(NQ - 1, -1, -1):
            pend.append((i, _scores(i, q_s, k_s)))
            if len(pend) > 1:
                pi, st = pend.pop(0)
                opend.append((pi, _context(pi, st, v_s)))
                if len(opend) > 1:
                    out_proj(*opend.pop(0))
        pi, st = pend.pop(0)
        opend.append((pi, _context(pi, st, v_s)))
        for o in opend:
            out_proj(*o)

        @pl.when(h < H - 1)
        def _():
            k_s[...] = _dot(ckv[...], wukT[h + 1]).astype(BF16)
            q_s[...] = (_dot(x_s[...], wqT[h + 1]) * qscale).astype(BF16)

        return carry

    lax.fori_loop(0, H, head_body, 0)


@jax.jit
def pallas_gated_mix__compressed_kv_cla__linear_attn_block__prompt_kernel(
    A_x: jax.Array,
    A_c_kv: jax.Array,
    A_w_q: jax.Array,
    A_w_uk: jax.Array,
    A_w_uv: jax.Array,
    A_w_o: jax.Array,
    B_x: jax.Array,
    B_wqkv: jax.Array,
    B_wo: jax.Array,
    gate_w: jax.Array,
):
    del B_x
    hbm = pl.BlockSpec(memory_space=pltpu.HBM)
    outT = pl.pallas_call(
        kernel,
        out_shape=jax.ShapeDtypeStruct((M, S), BF16),
        in_specs=[hbm] * 8 + [pl.BlockSpec((M,), lambda: (0,))],
        out_specs=pl.BlockSpec((M, S), lambda: (0, 0)),
        scratch_shapes=[
            pltpu.VMEM((M, S), BF16),
            pltpu.VMEM((S, DC), BF16),
            pltpu.VMEM((M, H, D), BF16),
            pltpu.VMEM((DC, H, D), BF16),
            pltpu.VMEM((DC, H, D), BF16),
            pltpu.VMEM((H, M, D), BF16),
            pltpu.VMEM((M, 3 * M), BF16),
            pltpu.VMEM((M, M), BF16),
            pltpu.VMEM((S, M), BF16),
            pltpu.VMEM((H, M, D), BF16),
            pltpu.VMEM((H, DC, D), BF16),
            pltpu.VMEM((H, DC, D), BF16),
            pltpu.VMEM((S, D), BF16),
            pltpu.VMEM((S, D), BF16),
            pltpu.VMEM((S, D), BF16),
            pltpu.VMEM((M, S), BF16),
            pltpu.VMEM((8, S), F32),
            pltpu.VMEM((M, S), F32),
            pltpu.VMEM((2 * M + 16, M), BF16),
            pltpu.VMEM((M, M), F32),
            pltpu.VMEM((M, 128), F32),
            pltpu.VMEM((M, M), BF16),
            pltpu.VMEM((H, S), F32),
            pltpu.SemaphoreType.DMA((6 + 2 * WCH + NCB,)),
        ],
        compiler_params=pltpu.CompilerParams(vmem_limit_bytes=110 * 2**20),
        name="gmk",
    )(A_x[0].T, A_c_kv[0], A_w_q, A_w_uk, A_w_uv, A_w_o.transpose(0, 2, 1),
      B_wqkv, B_wo, gate_w)
    return outT.T[None]
```
